```python
import os as _os
_os.environ.setdefault("JAX_PLATFORMS", "cpu")
import jax
import jax.numpy as jnp

def _softmax(x, axis=-1):
    return jax.nn.softmax(x, axis=axis)
def _gelu(x):
    return jax.nn.gelu(x, approximate=True)
def _silu(x):
    return jax.nn.silu(x)
def _sigmoid(x):
    return jax.nn.sigmoid(x)
def _layernorm(x, axis=-1, eps=1e-5):
    m = jnp.mean(x, axis=axis, keepdims=True)
    v = jnp.var(x, axis=axis, keepdims=True)
    return (x - m) / jnp.sqrt(v + eps)
def _scatter_add(tgt, idx, src, axis=0):
    return tgt.at[idx].add(src)
def _segment_sum(src, seg, n):
    return jax.ops.segment_sum(src, seg, n)
class _Rng:
    def __init__(self, key):
        self._k = key
    def _next(self):
        self._k, sub = jax.random.split(self._k)
        return sub
    def normal(self, shape):
        return jax.random.normal(self._next(), shape, dtype=jnp.bfloat16)
    def randint(self, lo, hi, shape):
        return jax.random.randint(self._next(), shape, lo, hi, dtype=jnp.int32)
    def uniform(self, shape, lo=0.0, hi=1.0):
        return jax.random.uniform(self._next(), shape, jnp.bfloat16, lo, hi)
    def permutation(self, n):
        return jax.random.permutation(self._next(), n)


kernel_name = 'gated_mix__sliding_block_cached__swiglu_ffn__decode'

def setup_inputs():
    _rng = _Rng(jax.random.key(int.from_bytes(__import__("os").urandom(4), "little")))
    _w = (lambda a: (lambda t: t.astype(jnp.bfloat16) if jnp.issubdtype(t.dtype, jnp.floating) else t)(jnp.asarray(a)))
    def _A_setup():
        B, Sq, D = 1, 1, 512
        Hq, Hkv, Sk, Dh = 32, 32, 32768, 128
        assert Hq % Hkv == 0, (Hq, Hkv)
        return {
            "x": _w((lambda *s: _rng.normal(s) * 0.05)(B, Sq, D)),
            "k_cache": _w((lambda *s: _rng.normal(s) * 3.2)(B, Hkv, Sk, Dh)),
            "v_cache": _w((lambda *s: _rng.normal(s) * 1.6)(B, Hkv, Sk, Dh)),
            "wq": _w((lambda *s: _rng.normal(s) * 3.2)(D, Hq * Dh) * (D ** -0.5)),
            "wo": _w((lambda *s: _rng.normal(s) * 1.6)(Hq * Dh, D) * ((Hq * Dh) ** -0.5)),
        }
    _A_in = _A_setup()

    def _B_setup():
        B, S, D, F = 1, 1, 512, 1376
        return {
            "x": _w((lambda *s: _rng.normal(s) * 0.05)(B, S, D)),
            "w_gate": _w((lambda *s: _rng.normal(s) * 0.1)(D, F)),
            "w_up": _w((lambda *s: _rng.normal(s) * 0.1)(D, F)),
            "w_down": _w((lambda *s: _rng.normal(s) * 0.1)(F, D)),
        }
    _B_in = _B_setup()

    return {
        "A_x": _A_in["x"],
        "A_k_cache": _A_in["k_cache"],
        "A_v_cache": _A_in["v_cache"],
        "A_wq": _A_in["wq"],
        "A_wo": _A_in["wo"],
        "B_x": _B_in["x"],
        "B_w_gate": _B_in["w_gate"],
        "B_w_up": _B_in["w_up"],
        "B_w_down": _B_in["w_down"],
        "gate_w": _w((lambda *s: _rng.normal(s) * 0.05)(512) * 16.0),
    }

def reference(A_x, A_k_cache, A_v_cache, A_wq, A_wo, B_x, B_w_gate, B_w_up, B_w_down, gate_w):
    def _A_ref(x, k_cache, v_cache, wq, wo):
        B, Sq, D = x.shape
        Hq, Dh = 32, 128
        Hkv, Sk = k_cache.shape[1], k_cache.shape[2]
        W = min(4096, max(256, Sk // 4))
        rep = Hq // Hkv
        q = (lambda x, *d: x.transpose(*d))((x @ wq).reshape(B, Sq, Hq, Dh), 0, 2, 1, 3)
        k = jnp.repeat(k_cache[:, :, Sk - W:, :], rep, axis=1)
        v = jnp.repeat(v_cache[:, :, Sk - W:, :], rep, axis=1)
        scores = jnp.einsum("bhqd,bhkd->bhqk", q, k) * (Dh ** -0.5)
        p = _softmax(scores, axis=-1)
        o = jnp.einsum("bhqk,bhkd->bhqd", p, v)
        return (lambda x, *d: x.transpose(*d))(o, 0, 2, 1, 3).reshape(B, Sq, Hq * Dh) @ wo

    def _B_ref(x, w_gate, w_up, w_down):
        g = _silu(x @ w_gate)
        u = x @ w_up
        return (g * u) @ w_down

    x = A_x
    g = _sigmoid((x * gate_w).sum(-1, keepdims=True))
    a = _A_ref(x, A_k_cache, A_v_cache, A_wq, A_wo)
    b = _B_ref(x, B_w_gate, B_w_up, B_w_down)
    return g * a + (1 - g) * b
```

```python
import functools

import jax
import jax.numpy as jnp
from jax import lax
from jax.experimental import pallas as pl
from jax.experimental.pallas import tpu as pltpu

_HQ, _DH = 32, 128
_ROWS = 8
_NT = (((1,), (1,)), ((), ()))
_HI, _LO = 0, 1


def _split(total, n, unit):
    u = total // unit
    assert u * unit == total
    cuts = [unit * ((u * i) // n) for i in range(n + 1)]
    return [(a, b - a) for a, b in zip(cuts[:-1], cuts[1:])]


def _kernel(x_hbm, k_hbm, v_hbm, wq_hbm, wo_hbm, wg_hbm, wu_hbm, wd_hbm, gw_hbm,
            out_ref,
            x_v, gw_v, wq_v, wo_v, ffn_v, kv_v, q_s, o_s, b_s, sems, *, cfg):
    W = kv_v.shape[2]
    SK = k_hbm.shape[2]
    D, E = wq_v.shape
    F = ffn_v.shape[1]
    NB = kv_v.shape[0]
    S_X, S_WQ, S_FFN = NB, NB + 1, NB + 2

    def copy(src, dst, s):
        return pltpu.make_async_copy(src, dst, sems.at[s])

    def wq_piece(i):
        r = pl.multiple_of((i // 2) * 8, 8)
        c = pl.multiple_of((i % 2) * (E // 2), E // 2)
        copy(wq_hbm.at[pl.ds(r, 8), pl.ds(c, E // 2)], wq_v.at[pl.ds(r, 8), pl.ds(c, E // 2)], S_WQ).start(priority=_LO)

    def ffn_piece(w, i, prio):
        r = pl.multiple_of(i * 32, 32)
        copy((wg_hbm, wu_hbm, wd_hbm)[w].at[pl.ds(r, 32)], ffn_v.at[w, pl.ds(r, 32)], S_FFN).start(priority=prio)

    def loop(n, fn):
        def body(i, c):
            fn(i)
            return c
        lax.fori_loop(0, n, body, 0)

    nq = 2 * D // 8
    nf = F // 32
    lead = cfg["lead"]
    loop(lead, wq_piece)
    x_cp = copy(x_hbm, x_v, S_X)
    gw_cp = copy(gw_hbm, gw_v, S_X)
    x_cp.start()
    gw_cp.start()
    for w in range(2):
        def pair(i, w=w):
            ffn_piece(w, i, _HI)
            wq_piece(lead + w * nf + i)
        loop(nf, pair)
    rest = nq - lead - 2 * nf
    def pair(i):
        ffn_piece(2, i, _HI)
        wq_piece(lead + 2 * nf + i)
    loop(rest, pair)
    half = (nf - rest) // 2
    def pair(i):
        ffn_piece(2, rest + i, _HI)
        ffn_piece(2, nf - half + i, _LO)
    loop(half, pair)
    if rest + 2 * half < nf:
        ffn_piece(2, rest + half, _HI)

    kv_pieces = _split(W, cfg["nkv"], 16)

    def start_head(h):
        slot = h % NB
        for off, n in kv_pieces:
            for j, (src, prio) in enumerate(((k_hbm, _HI), (v_hbm, _LO))):
                copy(src.at[0, h, pl.ds(SK - W + off, n)], kv_v.at[slot, j, pl.ds(off, n)], slot).start(priority=prio)

    loop(2, start_head)

    x_cp.wait()
    gw_cp.wait()
    xf = x_v[0].astype(jnp.float32)
    x8 = jnp.broadcast_to(xf, (_ROWS, D)).astype(jnp.bfloat16)
    gwf = gw_v[...].astype(jnp.float32)
    z = sum(xf[:, 128 * i:128 * (i + 1)] * gwf[i:i + 1, :] for i in range(D // 128))
    gate = jax.nn.sigmoid(jnp.sum(z, axis=-1, keepdims=True))

    copy(ffn_v, ffn_v, S_FFN).wait()
    g = lax.dot_general(x8, ffn_v[0], _NT, preferred_element_type=jnp.float32)
    u = lax.dot_general(x8, ffn_v[1], _NT, preferred_element_type=jnp.float32)
    hid = (g * jax.nn.sigmoid(g) * u).astype(jnp.bfloat16)
    b = jnp.dot(hid, ffn_v[2], preferred_element_type=jnp.float32)
    b_s[...] = (1.0 - gate) * b

    copy(wq_v, wq_v, S_WQ).wait()
    q = jnp.dot(x8, wq_v[...], preferred_element_type=jnp.float32).astype(jnp.bfloat16)
    for h in range(_HQ):
        q_s[h] = q[:, h * _DH:(h + 1) * _DH]

    groups = cfg["wo_groups"]
    def wo_rows(first, n):
        return [(first * _DH + 32 * i, 32) for i in range(n * _DH // 32)]
    hi = [(r, n, groups[0][2]) for r, n in wo_rows(*groups[0][:2])]
    lo = [(r, n, s) for f, c, s in groups[1:] for r, n in wo_rows(f, c)]
    order = []
    for i in range(max(len(hi), len(lo))):
        if i < len(hi): order.append(hi[i] + (_HI,))
        if i < len(lo): order.append(lo[i] + (_LO,))
    def start_wo(part):
        m = len(order) // 2
        for r, n, s, prio in (order[:m], order[m:])[part]:
            copy(wo_hbm.at[pl.ds(r, n)], wo_v.at[pl.ds(r, n)], s).start(priority=prio)

    def head(h):
        pl.when(h < _HQ - 2)(lambda: start_head(h + 2))
        pl.when(h == _HQ - 2)(lambda: start_wo(0))
        pl.when(h == _HQ - 1)(lambda: start_wo(1))
        slot = h % NB
        copy(kv_v.at[slot], kv_v.at[slot], slot).wait()
        s = lax.dot_general(q_s[h], kv_v[slot, 0], _NT, preferred_element_type=jnp.float32) * (_DH ** -0.5)
        m = jnp.max(s, axis=-1, keepdims=True)
        p = jnp.exp(s - m)
        l = jnp.sum(p, axis=-1, keepdims=True)
        o = jnp.dot(p.astype(jnp.bfloat16), kv_v[slot, 1], preferred_element_type=jnp.float32)
        o_s[h] = (o / l).astype(jnp.bfloat16)

    loop(_HQ, head)

    a = None
    for first, n, s in groups:
        rows = wo_v.at[pl.ds(first * _DH, n * _DH)]
        copy(rows, rows, s).wait()
        o_cat = jnp.concatenate([o_s[first + i] for i in range(n)], axis=-1)
        part = jnp.dot(o_cat, rows[...], preferred_element_type=jnp.float32)
        a = part if a is None else a + part
    res = gate * a + b_s[...]
    out_ref[0] = res[0:1, :].astype(out_ref.dtype)


def build(cfg):
    def fn(A_x, A_k_cache, A_v_cache, A_wq, A_wo, B_x, B_w_gate, B_w_up, B_w_down, gate_w):
        del B_x
        D = A_x.shape[-1]
        SK = A_k_cache.shape[2]
        W = min(4096, max(256, SK // 4))
        F = B_w_down.shape[0]
        NB = 4
        bf = jnp.bfloat16
        hbm = pl.BlockSpec(memory_space=pltpu.HBM)
        return pl.pallas_call(
            functools.partial(_kernel, cfg=cfg),
            in_specs=[hbm] * 9,
            out_specs=pl.BlockSpec(memory_space=pltpu.VMEM),
            out_shape=jax.ShapeDtypeStruct(A_x.shape, A_x.dtype),
            scratch_shapes=[
                pltpu.VMEM(A_x.shape, bf),
                pltpu.VMEM((D // 128, 128), bf),
                pltpu.VMEM(A_wq.shape, bf),
                pltpu.VMEM(A_wo.shape, bf),
                pltpu.VMEM((3, F, D), bf),
                pltpu.VMEM((NB, 2, W, _DH), bf),
                pltpu.VMEM((_HQ, _ROWS, _DH), bf),
                pltpu.VMEM((_HQ, _ROWS, _DH), bf),
                pltpu.VMEM((_ROWS, D), jnp.float32),
                pltpu.SemaphoreType.DMA((NB + 3,)),
            ],
            compiler_params=pltpu.CompilerParams(vmem_limit_bytes=48 * 1024 * 1024, **cfg.get("cp", {})),
            name="gated_mix_decode",
        )(A_x, A_k_cache, A_v_cache, A_wq, A_wo, B_w_gate.T, B_w_up.T, B_w_down, gate_w.reshape(D // 128, 128))
    return jax.jit(fn)

DEFAULT = dict(lead=32, nkv=24, wo_groups=[(0, 16, 4), (16, 12, 5), (28, 3, 6), (31, 1, 0)])


@jax.jit
def pallas_gated_mix__sliding_block_cached__swiglu_ffn__decode_kernel(
    A_x, A_k_cache, A_v_cache, A_wq, A_wo, B_x, B_w_gate, B_w_up, B_w_down, gate_w):
    return build(DEFAULT)(A_x, A_k_cache, A_v_cache, A_wq, A_wo, B_x, B_w_gate, B_w_up, B_w_down, gate_w)
```

```python
import functools

import jax
import jax.numpy as jnp
from jax import lax
from jax.experimental import pallas as pl
from jax.experimental.pallas import tpu as pltpu

_HQ, _DH = 32, 128
_ROWS = 8
_NT = (((1,), (1,)), ((), ()))
_HI, _LO = 0, 1

_GROUP = 8
_N_GROUPS = _HQ // _GROUP
_PAIR = 2
_KV_RUN = 64
_W_RUN = 16
_BURST = 32
_LAG = 3
_LO_LEAD = 32
_LO_DELAY = 28
_BANDS = 8
_SLOTS = _HQ // _BANDS

_S_X, _S_GATE, _S_WQ, _S_FFN, _S_WO = range(_N_GROUPS, _N_GROUPS + 5)
_N_SEMS = _S_WO + _SLOTS + 1


def _loop(start, stop, fn):
    def body(i, carry):
        fn(i)
        return carry

    lax.fori_loop(start, stop, body, 0)


def _aligned(v, m):
    return v if isinstance(v, int) else pl.multiple_of(v, m)


def _interleave(a, b):
    keyed = [((i + 0.5) / len(xs), w, i) for w, xs in enumerate((a, b)) for i in range(len(xs))]
    return [(a, b)[w][i] for _, w, i in sorted(keyed)]


def _body(x_hbm, k_hbm, v_hbm, wq_hbm, wo_hbm, wg_hbm, wu_hbm, wd_hbm, gate_hbm,
          out_ref,
          x_v, gate_v, wq_v, wo_v, ffn_v, kv_v, x_s, q_s, o_s, gate_s, acc_s, sems):
    f32, bf16 = jnp.float32, jnp.bfloat16
    Sk, W = k_hbm.shape[2], kv_v.shape[3]
    D, E = wq_v.shape
    F = ffn_v.shape[1] * ffn_v.shape[2]

    def copy(src, dst, sem):
        return pltpu.make_async_copy(src, dst, sems.at[sem])

    def fetch(src, dst, idx, sem, priority):
        copy(src.at[idx], dst.at[idx], sem).start(priority=priority)

    def wait_filled(buf, sem):
        copy(buf, buf, sem).wait()

    wq_cols = 4
    n_wq = D // _W_RUN * wq_cols

    def fetch_wq(i, priority):
        band, col, row = i % _BANDS, i // _BANDS % wq_cols, i // (_BANDS * wq_cols)
        rows = pl.ds(_aligned(band * (D // _BANDS) + row * _W_RUN, _W_RUN), _W_RUN)
        cols = pl.ds(_aligned(col * (E // wq_cols), E // wq_cols), E // wq_cols)
        fetch(wq_hbm, wq_v, (rows, cols), _S_WQ, priority)

    n_runs = W // _KV_RUN
    runs_per_step = _BURST // _GROUP
    steps = n_runs // runs_per_step
    assert (n_wq - _LO_LEAD) // 2 <= n_runs and _LAG + _GROUP // _PAIR <= steps

    def fetch_kv(t):
        g = t // steps

        def run(p):
            off = pl.multiple_of((p - g * n_runs) * _KV_RUN, _KV_RUN)
            for j in range(0, _GROUP, 2):
                for kv, (src, priority) in enumerate(((k_hbm, _HI), (v_hbm, _LO))):
                    copy(src.at[0, pl.ds(g * _GROUP + j, 2), pl.ds(Sk - W + off, _KV_RUN)],
                         kv_v.at[g, kv, pl.ds(j, 2), pl.ds(off, _KV_RUN)], g).start(priority=priority)

            @pl.when(p < (n_wq - _LO_LEAD) // 2)
            def _():
                fetch_wq(_LO_LEAD + 2 * p, _HI)
                fetch_wq(_LO_LEAD + 2 * p + 1, _LO)

        _loop(t * runs_per_step, (t + 1) * runs_per_step, run)

    last = _SLOTS - 1
    ffn = [(src, ffn_v.at[w], (slice(None), pl.ds(r, _W_RUN)), _S_FFN)
           for r in range(0, F // 2, _W_RUN) for w, src in enumerate((wg_hbm, wu_hbm, wd_hbm))]
    wo = [(wo_hbm, wo_v, (pl.ds(band, 2), pl.ds(r, _W_RUN)), _S_WO + r // _DH)
          for r in range(0, _SLOTS * _DH, _W_RUN) for band in range(0, _BANDS, 2)
          if r < last * _DH or band < _BANDS - 2]
    wo_end = [(wo_hbm, wo_v, (band, pl.ds(r, _W_RUN), pl.ds(c, D // 2)), _S_WO + _SLOTS)
              for r in range(last * _DH, _SLOTS * _DH, _W_RUN) for c in (0, D // 2)
              for band in (_BANDS - 2, _BANDS - 1)]
    early = 2 * len(wo) // 5
    landing = _interleave(ffn, wo[:early]) + wo[early:]
    queues = (landing[:_LO_DELAY] + landing[_LO_DELAY::2], landing[_LO_DELAY + 1::2] + wo_end)
    tail = [q[i] + (priority,) for i in range(max(map(len, queues)))
            for priority, q in zip((_HI, _LO), queues) if i < len(q)]

    def fetch_tail(copies):
        for args in copies:
            fetch(*args)

    x_copy = copy(x_hbm, x_v, _S_X)
    gate_copy = copy(gate_hbm, gate_v, _S_GATE)

    def gate_and_q():
        x_copy.wait()
        gate_copy.wait()
        x = x_v[0].astype(f32)
        x_s[...] = jnp.broadcast_to(x, (_ROWS, D)).astype(bf16)
        gw = gate_v[...].astype(f32)
        z = sum(x[:, 128 * i:128 * (i + 1)] * gw[i:i + 1, :] for i in range(D // 128))
        gate = jax.nn.sigmoid(jnp.sum(z, axis=-1, keepdims=True))
        gate_s[...] = jnp.broadcast_to(gate, (_ROWS, D))

        wait_filled(wq_v, _S_WQ)

        def project(g):
            cols = pl.ds(pl.multiple_of(g * _GROUP * _DH, _GROUP * _DH), _GROUP * _DH)
            q = jnp.dot(x_s[...], wq_v[:, cols], preferred_element_type=f32).astype(bf16)
            for j in range(_GROUP):
                q_s[g * _GROUP + j] = q[:, j * _DH:(j + 1) * _DH]

        _loop(0, _N_GROUPS, project)

    def attend(g, i):
        pl.when(i == 0)(lambda: wait_filled(kv_v.at[g], g))
        heads = [i * _PAIR + j for j in range(_PAIR)]
        scores = [lax.dot_general(q_s[g * _GROUP + h], kv_v[g, 0, h], _NT,
                                  preferred_element_type=f32) * (_DH ** -0.5) for h in heads]
        for h, s in zip(heads, scores):
            p = jnp.exp(s - jnp.max(s, axis=-1, keepdims=True))
            o = jnp.dot(p.astype(bf16), kv_v[g, 1, h], preferred_element_type=f32)
            o_s[g * _GROUP + h] = (o / jnp.sum(p, axis=-1, keepdims=True)).astype(bf16)

    def mix_in_heads(first_band, n_bands, slot, sem):
        rows = pl.ds(_aligned(slot * _DH, _DH), _DH)
        wait_filled(wo_v.at[pl.ds(first_band, n_bands), rows], sem)
        a = sum(jnp.dot(o_s[band * _SLOTS + slot], wo_v[band, rows, :], preferred_element_type=f32)
                for band in range(first_band, first_band + n_bands))
        return acc_s[...] + gate_s[...] * a

    for i in range(_LO_LEAD):
        fetch_wq(i, _LO)
    x_copy.start()
    gate_copy.start()

    kv_steps = _N_GROUPS * steps
    tail_steps = _LAG + _GROUP // _PAIR

    def step(t):
        pl.when(t < kv_steps)(lambda: fetch_kv(t))

        @pl.when(t >= kv_steps)
        def _():
            for k in range(tail_steps):
                pl.when(t == kv_steps + k)(functools.partial(fetch_tail, tail[k * _BURST:(k + 1) * _BURST]))

        pl.when(t == steps)(gate_and_q)
        i = t % steps - _LAG
        pl.when((t >= steps) & (i >= 0) & (i < _GROUP // _PAIR))(lambda: attend(t // steps - 1, i))

    _loop(0, kv_steps + tail_steps, step)
    fetch_tail(tail[tail_steps * _BURST:])

    wait_filled(ffn_v, _S_FFN)
    x = x_s[...]
    g = lax.dot_general(x, ffn_v[0].reshape(F, D), _NT, preferred_element_type=f32)
    u = lax.dot_general(x, ffn_v[1].reshape(F, D), _NT, preferred_element_type=f32)
    hidden = (g * jax.nn.sigmoid(g) * u).astype(bf16)
    b = jnp.dot(hidden, ffn_v[2].reshape(F, D), preferred_element_type=f32)
    acc_s[...] = (1.0 - gate_s[...]) * b

    def mix_in_slot(slot):
        acc_s[...] = mix_in_heads(0, _BANDS, slot, _S_WO + slot)

    _loop(0, last, mix_in_slot)
    acc_s[...] = mix_in_heads(0, _BANDS - 2, last, _S_WO + last)
    out = mix_in_heads(_BANDS - 2, 2, last, _S_WO + _SLOTS)
    out_ref[0] = out[0:1, :].astype(out_ref.dtype)


def _kernel(*refs):
    pl.run_scoped(functools.partial(_body, *refs), pltpu.SemaphoreType.DMA((_N_SEMS,)))


@jax.jit
def pallas_gated_mix__sliding_block_cached__swiglu_ffn__decode_kernel(
    A_x: jax.Array,
    A_k_cache: jax.Array,
    A_v_cache: jax.Array,
    A_wq: jax.Array,
    A_wo: jax.Array,
    B_x: jax.Array,
    B_w_gate: jax.Array,
    B_w_up: jax.Array,
    B_w_down: jax.Array,
    gate_w: jax.Array,
):
    del B_x
    B, Sq, D = A_x.shape
    _, Hkv, Sk, Dh = A_k_cache.shape
    F = B_w_down.shape[0]
    E = _HQ * _DH
    W = min(4096, max(256, Sk // 4))
    assert (B, Sq, Hkv, Dh) == (1, 1, _HQ, _DH)
    assert D % 256 == 0 and F % (2 * _W_RUN) == 0 and W % (_KV_RUN * _BURST // _GROUP) == 0

    bf16, f32 = jnp.bfloat16, jnp.float32
    return pl.pallas_call(
        _kernel,
        in_specs=[pl.BlockSpec(memory_space=pltpu.HBM)] * 9,
        out_specs=pl.BlockSpec(memory_space=pltpu.VMEM),
        out_shape=jax.ShapeDtypeStruct(A_x.shape, A_x.dtype),
        scratch_shapes=[
            pltpu.VMEM((1, 1, D), bf16),
            pltpu.VMEM((D // 128, 128), bf16),
            pltpu.VMEM((D, E), bf16),
            pltpu.VMEM((_BANDS, E // _BANDS, D), bf16),
            pltpu.VMEM((3, 2, F // 2, D), bf16),
            pltpu.VMEM((_N_GROUPS, 2, _GROUP, W, _DH), bf16),
            pltpu.VMEM((_ROWS, D), bf16),
            pltpu.VMEM((_HQ, _ROWS, _DH), bf16),
            pltpu.VMEM((_HQ, _ROWS, _DH), bf16),
            pltpu.VMEM((_ROWS, D), f32),
            pltpu.VMEM((_ROWS, D), f32),
        ],
        compiler_params=pltpu.CompilerParams(vmem_limit_bytes=96 * 1024 * 1024),
    )(
        A_x, A_k_cache, A_v_cache, A_wq,
        A_wo.reshape(_BANDS, E // _BANDS, D),
        B_w_gate.T.reshape(2, F // 2, D),
        B_w_up.T.reshape(2, F // 2, D),
        B_w_down.reshape(2, F // 2, D),
        gate_w.reshape(D // 128, 128),
    )
```
